```python
import os as _os
_os.environ.setdefault("JAX_PLATFORMS", "cpu")
import jax
import jax.numpy as jnp

def _softmax(x, axis=-1):
    return jax.nn.softmax(x, axis=axis)
def _gelu(x):
    return jax.nn.gelu(x, approximate=True)
def _silu(x):
    return jax.nn.silu(x)
def _sigmoid(x):
    return jax.nn.sigmoid(x)
def _layernorm(x, axis=-1, eps=1e-5):
    m = jnp.mean(x, axis=axis, keepdims=True)
    v = jnp.var(x, axis=axis, keepdims=True)
    return (x - m) / jnp.sqrt(v + eps)
def _scatter_add(tgt, idx, src, axis=0):
    return tgt.at[idx].add(src)
def _segment_sum(src, seg, n):
    return jax.ops.segment_sum(src, seg, n)
class _Rng:
    def __init__(self, key):
        self._k = key
    def _next(self):
        self._k, sub = jax.random.split(self._k)
        return sub
    def normal(self, shape):
        return jax.random.normal(self._next(), shape, dtype=jnp.bfloat16)
    def randint(self, lo, hi, shape):
        return jax.random.randint(self._next(), shape, lo, hi, dtype=jnp.int32)
    def uniform(self, shape, lo=0.0, hi=1.0):
        return jax.random.uniform(self._next(), shape, jnp.bfloat16, lo, hi)
    def permutation(self, n):
        return jax.random.permutation(self._next(), n)


kernel_name = 'sequential_preLN__sliding_block__dense_activation_gelu__prompt'

def setup_inputs():
    _rng = _Rng(jax.random.key(int.from_bytes(__import__("os").urandom(4), "little")))
    _w = (lambda a: (lambda t: t.astype(jnp.bfloat16) if jnp.issubdtype(t.dtype, jnp.floating) else t)(jnp.asarray(a)))
    def _A_setup():
        B, S, D = 1, 2048, 640
        return {
            "x": _w((lambda *s: _rng.normal(s) * 0.05)(B, S, D)),
            "wqkv": _w((lambda *s: _rng.normal(s) * 0.05)(D, 3 * D)),
            "wo": _w((lambda *s: _rng.normal(s) * 0.05)(D, D)),
        }
    _A_in = _A_setup()

    def _B_setup():
        B, S, D, F = 1, 2048, 640, 1536
        return {
            "x": _w((lambda *s: _rng.normal(s) * 0.05)(B, S, D)),
            "w1": _w((lambda *s: _rng.normal(s) * 0.8)(D, F) * (D ** -0.5)),
            "b1": _w((lambda *s: _rng.normal(s) * 0.8)(F) * 0.01),
            "w2": _w((lambda *s: _rng.normal(s) * 0.8)(F, D) * (F ** -0.5)),
            "b2": _w((lambda *s: _rng.normal(s) * 0.05)(D) * 0.01),
        }
    _B_in = _B_setup()

    return {
        "A_x": _A_in["x"],
        "A_wqkv": _A_in["wqkv"],
        "A_wo": _A_in["wo"],
        "B_x": _B_in["x"],
        "B_w1": _B_in["w1"],
        "B_b1": _B_in["b1"],
        "B_w2": _B_in["w2"],
        "B_b2": _B_in["b2"],
    }

def reference(A_x, A_wqkv, A_wo, B_x, B_w1, B_b1, B_w2, B_b2):
    def _A_ref(x, wqkv, wo):
        B, S, D = x.shape
        H = 32; Dh = D // H; W = 256
        qkv = (lambda x, *d: x.transpose(*d))((x @ wqkv).reshape(B, S, 3, H, Dh), 2, 0, 3, 1, 4)
        q, k, v = qkv[0], qkv[1], qkv[2]
        scores = jnp.einsum("bhqd,bhkd->bhqk", q, k) * (Dh ** -0.5)
        idx = jnp.arange(S)
        mask = (idx[:, None] - idx[None, :] >= 0) & (idx[:, None] - idx[None, :] < W)
        scores = jnp.where(mask[None, None], scores, -1e9)
        p = _softmax(scores, axis=-1)
        o = jnp.einsum("bhqk,bhkd->bhqd", p, v)
        return (lambda x, *d: x.transpose(*d))(o, 0, 2, 1, 3).reshape(B, S, D) @ wo

    def _B_ref(x, w1, b1, w2, b2):
        h = jnp.einsum("bsd,df->bsf", x, w1) + b1
        h = _gelu(h)
        return jnp.einsum("bsf,fd->bsd", h, w2) + b2

    x = A_x
    h = x + _A_ref(_layernorm(x, axis=-1), A_wqkv, A_wo)
    h2 = h + _B_ref(_layernorm(h, axis=-1), B_w1, B_b1, B_w2, B_b2)
    return h2
```

```python
import functools
import math
import jax
import jax.numpy as jnp
from jax import lax
import jax.experimental.pallas as pl
import jax.experimental.pallas.tpu as pltpu

S, D, H, DH, W, F = 2048, 640, 32, 20, 256, 1536
TQ = 128
T = 256
NQ = T // TQ
GH = 4
NTILES = S // TQ + 2
EPS = 1e-5
QSCALE = (DH ** -0.5) * math.log2(math.e)
NT = (((1,), (1,)), ((), ()))
f32 = jnp.float32
bf16 = jnp.bfloat16


def _ln(x):
    m = jnp.mean(x, axis=-1, keepdims=True)
    xc = x - m
    v = jnp.mean(xc * xc, axis=-1, keepdims=True)
    return xc * lax.rsqrt(v + EPS)


def _gelu(x):
    c = math.sqrt(2.0 / math.pi)
    return 0.5 * x * (1.0 + jnp.tanh(c * (x + 0.044715 * (x * x * x))))


def kernel(x_ref, wqkv_ref, wo_ref, w1_ref, b1_ref, w2_ref, b2_ref, o_ref,
           k_scr, vt_scr, q_scr, ot_scr):
    s = pl.program_id(0)

    @pl.when(s == 0)
    def _():
        k_scr[0:2 * TQ, :] = jnp.zeros((2 * TQ, D), bf16)
        vt_scr[0] = jnp.zeros((D, TQ), bf16)
        vt_scr[1] = jnp.zeros((D, TQ), bf16)

    x = x_ref[...].astype(f32)
    xn = _ln(x).astype(bf16)
    q = jnp.dot(xn, wqkv_ref[:, 0:D], preferred_element_type=f32)
    q_scr[...] = (q * QSCALE).astype(bf16)
    k = jnp.dot(xn, wqkv_ref[:, D:2 * D], preferred_element_type=f32)
    row0 = pl.multiple_of(s * T + 2 * TQ, TQ)
    k_scr[pl.ds(row0, T), :] = k.astype(bf16)
    v = jnp.dot(xn, wqkv_ref[:, 2 * D:3 * D], preferred_element_type=f32)
    for j in range(NQ):
        vt_scr[s * NQ + j + 2] = v[j * TQ:(j + 1) * TQ, :].T.astype(bf16)

    kk = lax.broadcasted_iota(jnp.int32, (3 * TQ, TQ), 0)
    qq = lax.broadcasted_iota(jnp.int32, (3 * TQ, TQ), 1)
    biases = []
    for j in range(NQ):
        I = s * NQ + j
        d = 2 * TQ + qq - kk
        valid = (d >= 0) & (d < W) & (kk + (I - 2) * TQ >= 0)
        biases.append(jnp.where(valid, 0.0, -1e9).astype(f32))

    def stage_a(j, h):
        I = s * NQ + j
        krow0 = pl.multiple_of(I * TQ, TQ)
        c0 = h * DH
        g = c0 // 128
        g1 = (c0 + DH - 1) // 128
        wdt = (g1 - g + 1) * 128
        lo = c0 - g * 128
        qh = q_scr[j * TQ:(j + 1) * TQ, g * 128:g * 128 + wdt]
        lane = lax.broadcasted_iota(jnp.int32, (TQ, wdt), 1)
        lm = (lane >= lo) & (lane < lo + DH)
        qm = jnp.where(lm, qh, jnp.zeros_like(qh))
        kw = k_scr[pl.ds(krow0, 3 * TQ), g * 128:g * 128 + wdt]
        st = lax.dot_general(kw, qm, NT, preferred_element_type=f32)
        st = st + biases[j]
        m = jnp.max(st, axis=0, keepdims=True)
        return st, m

    def stage_b(j, h, st, m):
        I = s * NQ + j
        c0 = h * DH
        p = jnp.exp2(st - m)
        l = jnp.sum(p, axis=0, keepdims=True)
        pb = p.astype(bf16)
        r0 = (c0 // 16) * 16
        vt = jnp.concatenate([vt_scr[I + t, r0:r0 + 32, :] for t in range(3)], axis=1)
        ot = jnp.dot(vt, pb, preferred_element_type=f32)
        ot = ot * (1.0 / l)
        off = c0 - r0
        ot_scr[c0:c0 + DH, j * TQ:(j + 1) * TQ] = ot[off:off + DH, :]

    groups = [[(j, h) for h in range(g0, g0 + GH)] for j in range(NQ) for g0 in range(0, H, GH)]
    nxt = [stage_a(*u) for u in groups[0]]
    for gi in range(len(groups)):
        cur = nxt
        if gi + 1 < len(groups):
            nxt = [stage_a(*u) for u in groups[gi + 1]]
        for u, (st, m) in zip(groups[gi], cur):
            stage_b(*u, st, m)

    o = ot_scr[...].T.astype(bf16)
    h1 = x + jnp.dot(o, wo_ref[...], preferred_element_type=f32)
    hn = _ln(h1).astype(bf16)
    u = jnp.dot(hn, w1_ref[...], preferred_element_type=f32) + b1_ref[...].astype(f32)
    u = _gelu(u).astype(bf16)
    y = jnp.dot(u, w2_ref[...], preferred_element_type=f32) + b2_ref[...].astype(f32)
    o_ref[...] = (h1 + y).astype(o_ref.dtype)


@jax.jit
def pallas_sequential_preLN__sliding_block__dense_activation_gelu__prompt_kernel(
    A_x, A_wqkv, A_wo, B_x, B_w1, B_b1, B_w2, B_b2):
    x = A_x.reshape(S, D)
    b1 = B_b1.reshape(1, F)
    b2 = B_b2.reshape(1, D)
    const = lambda i: (0, 0)
    out = pl.pallas_call(
        kernel,
        grid=(S // T,),
        in_specs=[
            pl.BlockSpec((T, D), lambda i: (i, 0)),
            pl.BlockSpec((D, 3 * D), const),
            pl.BlockSpec((D, D), const),
            pl.BlockSpec((D, F), const),
            pl.BlockSpec((1, F), const),
            pl.BlockSpec((F, D), const),
            pl.BlockSpec((1, D), const),
        ],
        out_specs=pl.BlockSpec((T, D), lambda i: (i, 0)),
        out_shape=jax.ShapeDtypeStruct((S, D), bf16),
        scratch_shapes=[
            pltpu.VMEM((NTILES * TQ, D), bf16),
            pltpu.VMEM((NTILES, D, TQ), bf16),
            pltpu.VMEM((T, D), bf16),
            pltpu.VMEM((D, T), f32),
        ],
        compiler_params=pltpu.CompilerParams(
            dimension_semantics=("arbitrary",),
            vmem_limit_bytes=100 * 1024 * 1024,
        ),
    )(x, A_wqkv, A_wo, B_w1, b1, B_w2, b2)
    return out.reshape(1, S, D)
```

```python
import functools
import math
import jax
import jax.numpy as jnp
from jax import lax
import jax.experimental.pallas as pl
import jax.experimental.pallas.tpu as pltpu

S, D, H, DH, W, F = 2048, 640, 32, 20, 256, 1536
TQ = 128
HQ = TQ // 2
T = 256
NQ = T // TQ
GH = 4
NG = H // GH
NTILES = NQ + 2
EPS = 1e-5
QSCALE = (DH ** -0.5) * math.log2(math.e)
NEG = -1e9
NT = (((1,), (1,)), ((), ()))
f32 = jnp.float32
bf16 = jnp.bfloat16
u32 = jnp.uint32


def _ln(x):
    m = jnp.mean(x, axis=-1, keepdims=True)
    xc = x - m
    v = jnp.mean(xc * xc, axis=-1, keepdims=True)
    return xc * lax.rsqrt(v + EPS)


def _gelu(x):
    c = math.sqrt(2.0 / math.pi)
    return 0.5 * x * (1.0 + jnp.tanh(c * (x + 0.044715 * (x * x * x))))


def _pack_halves(x):
    r = x.shape[0] // 2
    return pltpu.bitcast(pltpu.pack_elementwise([x[:r], x[r:]], packed_dtype=bf16), u32)


def _head_tile(h):
    c0 = h * DH
    g = c0 // 128
    if (c0 + DH - 1) // 128 == g:
        return False, g, c0 - g * 128
    return True, g, c0 - (g * 128 + 64)


def kernel(x_ref, xnext_ref, wqkv_hbm, wo_hbm, w1_hbm, b1_ref, w2_hbm, b2_ref, o_ref,
           wqkv_ref, wo_ref, w1_ref, w2_ref, sems,
           k_scr, ks_scr, vt_scr, q_scr, qs_scr, ot_scr, xt_scr, xs_scr):
    s = pl.program_id(0)

    def slab(i):
        return pltpu.make_async_copy(wqkv_hbm.at[:, i * D:(i + 1) * D], wqkv_ref.at[:, i * D:(i + 1) * D],
                                     sems.at[i])

    copies = {
        'k': slab(1), 'v': slab(2), 'q': slab(0),
        'wo': pltpu.make_async_copy(wo_hbm, wo_ref, sems.at[3]),
        'w1': pltpu.make_async_copy(w1_hbm, w1_ref, sems.at[4]),
        'w2': pltpu.make_async_copy(w2_hbm, w2_ref, sems.at[5]),
    }

    def body(first):
        kk = lax.broadcasted_iota(jnp.int32, (TQ, TQ), 0)
        qq = lax.broadcasted_iota(jnp.int32, (TQ, TQ), 1)
        upper = kk > qq
        r2 = lax.broadcasted_iota(jnp.int32, (HQ, TQ), 0)
        q2 = lax.broadcasted_iota(jnp.int32, (HQ, TQ), 1)
        mu = jnp.where(r2 > q2, 0xFFFF, 0) | jnp.where(r2 + HQ > q2, -65536, 0)
        mu = pltpu.bitcast(mu, u32)
        ml = ~mu

        st8 = {}

        def ln1_vals(xb):
            xu = pltpu.bitcast(xb, u32)
            xe = pltpu.unpack_elementwise(xu, index=0, packed_dtype=bf16, unpacked_dtype=f32)
            xo = pltpu.unpack_elementwise(xu, index=1, packed_dtype=bf16, unpacked_dtype=f32)
            xn = _ln(jnp.concatenate([xe, xo], axis=0))
            nat = pltpu.bitcast(_pack_halves(xn), bf16).astype(f32)
            return xn.astype(bf16), _pack_halves(nat)

        def ln1(z):
            xt, xs = ln1_vals(x_ref[z * TQ:(z + 1) * TQ, :])
            st8['xt', z] = xt
            st8['xs', z] = pltpu.bitcast(xs, bf16)

        def ln1_load():
            st8['xt', 0] = xt_scr[...]
            st8['xs', 0] = pltpu.bitcast(xs_scr[...], bf16)

        def ln1_next():
            xt, xs = ln1_vals(xnext_ref[...])
            xt_scr[...] = xt
            xs_scr[...] = xs

        def qkv(z, t0, t1):
            xn = st8['xs' if t0 >= 10 else 'xt', z]
            r = jnp.dot(xn, wqkv_ref[:, t0 * 128:t1 * 128], preferred_element_type=f32)
            for t in range(t0, t1):
                rt = r[:, (t - t0) * 128:(t - t0 + 1) * 128]
                if t < 5:
                    q_scr[z * HQ:(z + 1) * HQ, t * 128:(t + 1) * 128] = _pack_halves(rt * QSCALE)
                elif t < 10:
                    k_scr[(z + 2) * HQ:(z + 3) * HQ, (t - 5) * 128:(t - 4) * 128] = _pack_halves(rt)
                else:
                    vt_scr[z + 2, (t - 10) * 128:(t - 9) * 128, :] = rt.T.astype(bf16)
            if t1 == 5:
                qs_scr[z * HQ:(z + 1) * HQ, :] = q_scr[z * HQ:(z + 1) * HQ, 64:576]
            if t1 == 10:
                ks_scr[(z + 2) * HQ:(z + 3) * HQ, :] = k_scr[(z + 2) * HQ:(z + 3) * HQ, 64:576]

        def ntiles(j):
            return min(3, j + 1) if first else 3

        def stage_a1(j, h):
            nt = ntiles(j)
            sh, g, lo = _head_tile(h)
            qr, kr = (qs_scr, ks_scr) if sh else (q_scr, k_scr)
            lane = lax.broadcasted_iota(jnp.int32, (HQ, 128), 1)
            lm = pltpu.bitcast(jnp.where((lane >= lo) & (lane < lo + DH), -1, 0), u32)
            qm = pltpu.bitcast(qr[j * HQ:(j + 1) * HQ, g * 128:(g + 1) * 128] & lm, bf16)
            kw = pltpu.bitcast(kr[(j + 3 - nt) * HQ:(j + 3) * HQ, g * 128:(g + 1) * 128], bf16)
            st = lax.dot_general(kw, qm, NT, preferred_element_type=f32)
            lo_t = st[(nt - 1) * TQ:nt * TQ]
            sm = jnp.where(upper, st[0:TQ] if nt == 3 else NEG, lo_t)
            if nt == 1:
                return sm, None, jnp.max(sm, axis=0, keepdims=True)
            s1 = st[(nt - 2) * TQ:(nt - 1) * TQ]
            m = jnp.max(jnp.maximum(sm, s1), axis=0, keepdims=True)
            return sm, s1, m

        def stage_b1(j, h, sm, s1, m):
            pm = jnp.exp2(sm - m)
            if s1 is None:
                return _pack_halves(pm), None, jnp.sum(pm, axis=0, keepdims=True)
            p1 = jnp.exp2(s1 - m)
            l = jnp.sum(pm + p1, axis=0, keepdims=True)
            return _pack_halves(pm), _pack_halves(p1), l

        def stage_c1(j, h, pmu, p1u, l):
            nt = ntiles(j)
            c0 = h * DH
            if nt == 3:
                parts = [pmu & mu, p1u, pmu & ml]
            elif nt == 2:
                parts = [p1u, pmu]
            else:
                parts = [pmu]
            pb = jnp.concatenate([pltpu.bitcast(p, bf16) for p in parts], axis=0)
            r0 = (c0 // 16) * 16
            vt = jnp.concatenate([vt_scr[j + t, r0:r0 + 32, :] for t in range(3 - nt, 3)], axis=1)
            ot = jnp.dot(vt, pb, preferred_element_type=f32)
            ot = ot * (1.0 / l)
            off = c0 - r0
            ot_scr[c0:c0 + DH, j * TQ:(j + 1) * TQ] = ot[off:off + DH, :]

        def att_a(z, g):
            st8['s', z, g] = [stage_a1(z, h) for h in range(g * GH, (g + 1) * GH)]

        def att_b(z, g):
            hs = list(range(g * GH, (g + 1) * GH))
            ls = [stage_b1(z, h, *a) for h, a in zip(hs, st8.pop(('s', z, g)))]
            for h, l in zip(hs, ls):
                stage_c1(z, h, *l)

        def oproj(z):
            o = ot_scr[:, z * TQ:(z + 1) * TQ].T.astype(bf16)
            x = x_ref[z * TQ:(z + 1) * TQ, :].astype(f32)
            h1 = x + jnp.dot(o, wo_ref[...], preferred_element_type=f32)
            st8['h', z] = h1
            st8['hn', z] = _ln(h1).astype(bf16)

        def ffn1(z, c0, c1):
            u = jnp.dot(st8['hn', z], w1_ref[:, c0 * 128:c1 * 128], preferred_element_type=f32)
            u = u + b1_ref[:, c0 * 128:c1 * 128].astype(f32)
            st8['u', z, c0] = _gelu(u).astype(bf16)

        def ffn2(z, c0, c1):
            y = jnp.dot(st8.pop(('u', z, c0)), w2_ref[c0 * 128:c1 * 128, :], preferred_element_type=f32)
            st8['h', z] = st8['h', z] + y

        def fin(z):
            o_ref[z * TQ:(z + 1) * TQ, :] = (st8['h', z] + b2_ref[...].astype(f32)).astype(o_ref.dtype)

        def shift_hist():
            k_scr[0:2 * HQ, :] = k_scr[2 * HQ:4 * HQ, :]
            ks_scr[0:2 * HQ, :] = ks_scr[2 * HQ:4 * HQ, :]
            vt_scr[0] = vt_scr[2]
            vt_scr[1] = vt_scr[3]

        def wait(name):
            copies[name].wait()

        def run(item):
            if item is not None:
                item[0](*item[1:])

        if first:
            for name in ('k', 'v', 'q', 'wo', 'w1', 'w2'):
                copies[name].start()
            ln1(0)
            ln1(1)
            wait('k')
            qkv(0, 5, 10)
            qkv(1, 5, 10)
            wait('v')
            qkv(0, 10, 15)
            qkv(1, 10, 15)
            wait('q')
            qkv(0, 0, 5)
            att_a(0, 0)
            y0 = [(qkv, 1, 0, 2), None, (qkv, 1, 2, 5)] + [None] * 5
            y1 = [(wait, 'wo'), (oproj, 0), None, None, None, (wait, 'w1'), (ffn1, 0, 0, 4), (ffn1, 0, 4, 8)]
            tail = [(ffn1, 0, 8, 12), (oproj, 1), (shift_hist,), (wait, 'w2'), (ffn2, 0, 0, 4), (ffn2, 0, 4, 8),
                    (ffn2, 0, 8, 12), (fin, 0)]
        else:
            ln1_load()
            qkv(0, 5, 10)
            ln1(1)
            qkv(0, 10, 15)
            qkv(0, 0, 5)
            att_a(0, 0)
            y0 = [(qkv, 1, 5, 7), (qkv, 1, 7, 10), (qkv, 1, 10, 12), (qkv, 1, 12, 15), (qkv, 1, 0, 2),
                  (qkv, 1, 2, 5), None, None]
            y1 = [None, (oproj, 0), None, (ffn1, 0, 0, 4), None, (ffn1, 0, 4, 8), None, (ffn1, 0, 8, 12)]
            tail = [(ffn2, 0, 0, 4), (oproj, 1), (shift_hist,), (ffn2, 0, 4, 8), (ffn2, 0, 8, 12), (fin, 0)]
        for g in range(NG):
            if g + 1 < NG:
                att_a(0, g + 1)
            else:
                att_a(1, 0)
            run(y0[g])
            att_b(0, g)
        for g in range(NG):
            if g + 1 < NG:
                att_a(1, g + 1)
            run(y1[g])
            att_b(1, g)
        for item in tail:
            run(item)
        ffn1(1, 0, 4)
        ln1_next()
        ffn1(1, 4, 8)
        ffn2(1, 0, 4)
        ffn1(1, 8, 12)
        ffn2(1, 4, 8)
        ffn2(1, 8, 12)
        fin(1)

    @pl.when(s == 0)
    def _():
        body(True)

    @pl.when(s > 0)
    def _():
        body(False)


@jax.jit
def pallas_sequential_preLN__sliding_block__dense_activation_gelu__prompt_kernel(
    A_x, A_wqkv, A_wo, B_x, B_w1, B_b1, B_w2, B_b2):
    x = A_x.reshape(S, D)
    b1 = B_b1.reshape(1, F)
    b2 = B_b2.reshape(1, D)
    const = lambda i: (0, 0)
    hbm = pl.BlockSpec(memory_space=pl.ANY)
    out = pl.pallas_call(
        kernel,
        grid=(S // T,),
        in_specs=[
            pl.BlockSpec((T, D), lambda i: (i, 0)),
            pl.BlockSpec((TQ, D), lambda i: (jnp.minimum(NQ * (i + 1), S // TQ - 1), 0)),
            hbm, hbm, hbm,
            pl.BlockSpec((1, F), const),
            hbm,
            pl.BlockSpec((1, D), const),
        ],
        out_specs=pl.BlockSpec((T, D), lambda i: (i, 0)),
        out_shape=jax.ShapeDtypeStruct((S, D), bf16),
        scratch_shapes=[
            pltpu.VMEM((D, 3 * D), bf16),
            pltpu.VMEM((D, D), bf16),
            pltpu.VMEM((D, F), bf16),
            pltpu.VMEM((F, D), bf16),
            pltpu.SemaphoreType.DMA((6,)),
            pltpu.VMEM((NTILES * HQ, D), u32),
            pltpu.VMEM((NTILES * HQ, 512), u32),
            pltpu.VMEM((NTILES, D, TQ), bf16),
            pltpu.VMEM((NQ * HQ, D), u32),
            pltpu.VMEM((NQ * HQ, 512), u32),
            pltpu.VMEM((D, T), f32),
            pltpu.VMEM((TQ, D), bf16),
            pltpu.VMEM((HQ, D), u32),
        ],
        compiler_params=pltpu.CompilerParams(
            dimension_semantics=("arbitrary",),
            vmem_limit_bytes=100 * 1024 * 1024,
        ),
    )(x, x, A_wqkv, A_wo, B_w1, b1, B_w2, b2)
    return out.reshape(1, S, D)
```

```python
import math
import jax
import jax.numpy as jnp
from jax import lax
import jax.experimental.pallas as pl
import jax.experimental.pallas.tpu as pltpu

S, D, H, DH, W, F = 2048, 640, 32, 20, 256, 1536
TQ = 128
HQ = TQ // 2
T = 256
NQ = T // TQ
GH = 4
NG = H // GH
QN = TQ // GH
QW = QN // 2
NTILES = NQ + 2
EPS = 1e-5
QSCALE = (DH ** -0.5) * math.log2(math.e)
NEG = -1e9
LMAX = 2.0 ** 30
NT = (((1,), (1,)), ((), ()))
f32 = jnp.float32
bf16 = jnp.bfloat16
u32 = jnp.uint32
ONES2 = 0x3F803F80


def _ln(x):
    m = jnp.mean(x, axis=-1, keepdims=True)
    xc = x - m
    v = jnp.mean(xc * xc, axis=-1, keepdims=True)
    return xc * lax.rsqrt(v + EPS)


def _gelu(x):
    c = math.sqrt(2.0 / math.pi)
    return 0.5 * x * (1.0 + jnp.tanh(c * (x + 0.044715 * (x * x * x))))


def _pack_halves(x):
    r = x.shape[0] // 2
    return pltpu.bitcast(pltpu.pack_elementwise([x[:r], x[r:]], packed_dtype=bf16), u32)


def _pack16(x):
    n = x.shape[0] // 16
    a = jnp.concatenate([x[16 * k:16 * k + 8] for k in range(n)], axis=0)
    b = jnp.concatenate([x[16 * k + 8:16 * k + 16] for k in range(n)], axis=0)
    return pltpu.bitcast(pltpu.pack_elementwise([a, b], packed_dtype=bf16), u32)


def _group_tile(g):
    c0 = g * GH * DH
    t = c0 // 128
    if (c0 + GH * DH - 1) // 128 == t:
        return False, t, c0 - t * 128
    t = (c0 - 64) // 128
    assert c0 + GH * DH <= t * 128 + 192
    return True, t, c0 - (t * 128 + 64)


def kernel(x_hbm, wqkv_hbm, wo_hbm, w1_hbm, b1_hbm, w2_hbm, b2_hbm, o_ref,
           x_ref, wqkv_ref, wo_ref, w1_ref, b1_ref, w2_ref, b2_ref, sems, bad_ref,
           k_scr, ks_scr, vt_scr, q_scr, qs_scr, ot_scr, xt_scr, xs_scr):
    s = pl.program_id(0)

    def slab(i, sem):
        return pltpu.make_async_copy(wqkv_hbm.at[:, i * D:(i + 1) * D], wqkv_ref.at[:, i * D:(i + 1) * D],
                                     sems.at[sem])

    def xrows(r0, r1, sem):
        return pltpu.make_async_copy(x_hbm.at[r0:r1, :], x_ref.at[r0:r1, :], sems.at[sem])

    copies = {
        'q': slab(0, 0), 'k': slab(1, 1), 'v': slab(2, 2),
        'wo': pltpu.make_async_copy(wo_hbm, wo_ref, sems.at[3]),
        'w1': pltpu.make_async_copy(w1_hbm, w1_ref, sems.at[4]),
        'w2': pltpu.make_async_copy(w2_hbm, w2_ref, sems.at[5]),
        'b1': pltpu.make_async_copy(b1_hbm, b1_ref, sems.at[6]),
        'b2': pltpu.make_async_copy(b2_hbm, b2_ref, sems.at[7]),
        'xa': xrows(0, T, 8), 'xb': xrows(T, T + TQ, 9), 'xc': xrows(T + TQ, S, 10),
    }

    def body(mode):
        first, redo = mode == 'first', mode == 'redo'
        row0 = 0 if first else pl.multiple_of(s * T, T)

        ki = lax.broadcasted_iota(jnp.int32, (QN, TQ), 0)
        qi = lax.broadcasted_iota(jnp.int32, (QN, TQ), 1) & (QN - 1)
        tri = ki > qi
        if not first:
            r2 = lax.broadcasted_iota(jnp.int32, (HQ, TQ), 0)
            r2 = r2 + (r2 & -8)
            l2 = lax.broadcasted_iota(jnp.int32, (HQ, TQ), 1)
            mus, mls = [], []
            for a in range(GH):
                q2 = l2 ^ (QN * a)
                mu = jnp.where(r2 > q2, 0xFFFF, 0) | jnp.where(r2 + 8 > q2, -65536, 0)
                mu = pltpu.bitcast(mu, u32)
                mus.append(mu)
                mls.append(~mu)
        if redo:
            b0 = [jnp.where(s * NQ + j >= 2, 0.0, NEG).astype(f32) for j in range(NQ)]
            b1s = [jnp.where(s * NQ + j >= 1, 0.0, NEG).astype(f32) for j in range(NQ)]

        def butterfly(ts):
            lane = lax.broadcasted_iota(jnp.int32, ts[0].shape, 1)
            odd = (lane & QN) != 0
            us = [jnp.where(odd, ts[c ^ 1], ts[c]) for c in range(GH)]
            hi = (lane & (2 * QN)) != 0
            return [jnp.where(hi, us[a ^ 2], us[a]) for a in range(GH)]

        st8 = {'bad': jnp.zeros((1, TQ), f32)}

        def xblk(z):
            return x_ref[pl.ds(row0 + z * TQ, TQ), :]

        def ln1_vals(xb):
            xu = pltpu.bitcast(xb, u32)
            xe = pltpu.unpack_elementwise(xu, index=0, packed_dtype=bf16, unpacked_dtype=f32)
            xo = pltpu.unpack_elementwise(xu, index=1, packed_dtype=bf16, unpacked_dtype=f32)
            xn = _ln(jnp.concatenate([xe, xo], axis=0))
            nat = pltpu.bitcast(_pack_halves(xn), bf16).astype(f32)
            return xn.astype(bf16), _pack16(nat)

        def ln1(z):
            xt, xs = ln1_vals(xblk(z))
            st8['xt', z] = xt
            st8['xs', z] = pltpu.bitcast(xs, bf16)

        def ln1_load():
            st8['xt', 0] = xt_scr[...]
            st8['xs', 0] = pltpu.bitcast(xs_scr[...], bf16)

        def ln1_next():
            nxt = T if first else pl.multiple_of(jnp.minimum(row0 + T, S - TQ), TQ)
            xt, xs = ln1_vals(x_ref[pl.ds(nxt, TQ), :])
            xt_scr[...] = xt
            xs_scr[...] = xs

        def qkv(z, t0, t1):
            xn = st8['xs' if t0 >= 10 else 'xt', z]
            r = jnp.dot(xn, wqkv_ref[:, t0 * 128:t1 * 128], preferred_element_type=f32)
            for t in range(t0, t1):
                rt = r[:, (t - t0) * 128:(t - t0 + 1) * 128]
                if t < 5:
                    q_scr[z * HQ:(z + 1) * HQ, t * 128:(t + 1) * 128] = _pack_halves(rt * QSCALE)
                elif t < 10:
                    k_scr[(z + 2) * HQ:(z + 3) * HQ, (t - 5) * 128:(t - 4) * 128] = _pack_halves(rt)
                else:
                    vt_scr[z + 2, (t - 10) * 128:(t - 9) * 128, :] = rt.T.astype(bf16)
            if t1 == 5:
                qs_scr[z * HQ:(z + 1) * HQ, :] = q_scr[z * HQ:(z + 1) * HQ, 64:576]
            if t1 == 10:
                ks_scr[(z + 2) * HQ:(z + 3) * HQ, :] = k_scr[(z + 2) * HQ:(z + 3) * HQ, 64:576]

        def ntiles(j):
            return min(3, j + 1) if first else 3

        def stage_a1(j, g, c):
            nt = ntiles(j)
            sh, t, lo = _group_tile(g)
            qr, kr = (qs_scr, ks_scr) if sh else (q_scr, k_scr)
            lt = slice(t * 128, (t + 1) * 128)
            lane = lax.broadcasted_iota(jnp.int32, (QW, 128), 1)
            qc = qr[j * HQ + c * QW:j * HQ + (c + 1) * QW, lt]
            qs = []
            for lam in range(GH):
                l0 = lo + (lam ^ c) * DH
                lm = pltpu.bitcast(jnp.where((lane >= l0) & (lane < l0 + DH), -1, 0), u32)
                qs.append(qc & lm)
            qm = pltpu.bitcast(jnp.concatenate(qs, axis=0), bf16)
            d0 = (j + 2) * HQ + c * QW
            w0 = j * HQ + c * QW if nt == 3 else (j + 3 - nt) * HQ
            kw = kr[d0:d0 + QW, lt]
            if d0 > w0:
                kw = jnp.concatenate([kw, kr[w0:d0, lt]], axis=0)
            st = lax.dot_general(pltpu.bitcast(kw, bf16), qm, NT, preferred_element_type=f32)
            n = st.shape[0]
            parts = [st[n - QN * c:n]] if c > 0 else []
            if nt == 3:
                old = st[QN:TQ - QN * c + QN]
                if redo:
                    old = old + b0[j]
                parts.append(jnp.where(tri, old[0:QN], st[0:QN]))
                if c < GH - 1:
                    parts.append(old[QN:])
            else:
                parts.append(jnp.where(tri, NEG, st[0:QN]))
            sm = jnp.concatenate(parts, axis=0) if len(parts) > 1 else parts[0]
            s1 = st[n - QN * c - TQ:n - QN * c] if nt > 1 else None
            if redo:
                s1 = s1 + b1s[j]
                m = jnp.max(jnp.maximum(sm, s1), axis=0, keepdims=True)
            else:
                m = jnp.max(jnp.where(tri, NEG, st[0:QN]), axis=0, keepdims=True)
            return sm, s1, m

        def stage_b1(sm, s1, m):
            pm = jnp.exp2(sm - m)
            if pm.shape[0] < TQ:
                pm = jnp.concatenate([pm, jnp.zeros((TQ - pm.shape[0], TQ), f32)], axis=0)
            if s1 is None:
                return _pack16(pm), None
            return _pack16(pm), _pack16(jnp.exp2(s1 - m))

        def stage_c1(j, h, pmu, p1u):
            nt = ntiles(j)
            c0 = h * DH
            if nt == 3:
                parts = [pmu & mus[h % GH], p1u, pmu & mls[h % GH]]
            elif nt == 2:
                parts = [p1u, pmu]
            else:
                parts = [pmu]
            pb = jnp.concatenate([pltpu.bitcast(p, bf16) for p in parts], axis=0)
            r0 = (c0 // 16) * 16
            off = c0 - r0
            vt = jnp.concatenate([vt_scr[j + t, r0:r0 + 32, :] for t in range(3 - nt, 3)], axis=1)
            vu = pltpu.bitcast(vt, u32)
            wrow = lax.broadcasted_iota(jnp.int32, (8, nt * TQ), 0)
            if off < 12:
                lrow = 30
                vu = jnp.concatenate([vu[0:8], jnp.where(wrow == 7, jnp.uint32(ONES2), vu[8:16])], axis=0)
            else:
                lrow = 0
                vu = jnp.concatenate([jnp.where(wrow == 0, jnp.uint32(ONES2), vu[0:8]), vu[8:16]], axis=0)
            ot = jnp.dot(pltpu.bitcast(vu, bf16), pb, preferred_element_type=f32)
            l = ot[lrow:lrow + 1, :]
            if not redo:
                st8['bad'] = jnp.where(l <= LMAX, st8['bad'], 1.0)
            ot = ot * (1.0 / l)
            ot_scr[c0:c0 + DH, j * TQ:(j + 1) * TQ] = ot[off:off + DH, :]

        def att_a(z, g):
            st8['s', z, g] = [stage_a1(z, g, c) for c in range(GH)]

        def att_b(z, g):
            st8['p', z, g] = [stage_b1(*a) for a in st8.pop(('s', z, g))]

        def att_c(z, g):
            rs = st8.pop(('p', z, g))
            pms = butterfly([r[0] for r in rs])
            p1s = butterfly([r[1] for r in rs]) if rs[0][1] is not None else [None] * GH
            for a in range(GH):
                stage_c1(z, g * GH + a, pms[a], p1s[a])

        def oproj(z):
            o = ot_scr[:, z * TQ:(z + 1) * TQ].T
            if not redo:
                st8['fin', z] = jnp.sum(o - o, axis=0, keepdims=True)
            hid = lax.broadcasted_iota(jnp.int32, (QN, D), 1) // DH
            bs = [o[QN * i:QN * (i + 1)] for i in range(GH)]
            odd = (hid & 1) != 0
            us = [jnp.where(odd, bs[i ^ 1], bs[i]) for i in range(GH)]
            hi = (hid & 2) != 0
            o = jnp.concatenate([jnp.where(hi, us[i ^ 2], us[i]) for i in range(GH)], axis=0).astype(bf16)
            h1 = xblk(z).astype(f32) + jnp.dot(o, wo_ref[...], preferred_element_type=f32)
            st8['h', z] = h1
            st8['hn', z] = _ln(h1).astype(bf16)

        def biases():
            st8['b1'] = b1_ref[...].astype(f32).reshape(1, F)
            st8['b2'] = b2_ref[...].astype(f32).reshape(1, D)

        def ffn1(z, c0, c1):
            u = jnp.dot(st8['hn', z], w1_ref[:, c0 * 128:c1 * 128], preferred_element_type=f32)
            u = u + st8['b1'][:, c0 * 128:c1 * 128]
            st8['u', z, c0] = _gelu(u).astype(bf16)

        def ffn2(z, c0, c1):
            y = jnp.dot(st8.pop(('u', z, c0)), w2_ref[c0 * 128:c1 * 128, :], preferred_element_type=f32)
            st8['h', z] = st8['h', z] + y

        def fin(z):
            o_ref[z * TQ:(z + 1) * TQ, :] = (st8['h', z] + st8['b2']).astype(o_ref.dtype)

        def shift_hist():
            k_scr[0:2 * HQ, :] = k_scr[2 * HQ:4 * HQ, :]
            ks_scr[0:2 * HQ, :] = ks_scr[2 * HQ:4 * HQ, :]
            vt_scr[0] = vt_scr[2]
            vt_scr[1] = vt_scr[3]

        def zero_hist():
            k_scr[0:2 * HQ, :] = jnp.zeros((2 * HQ, D), u32)
            ks_scr[0:2 * HQ, :] = jnp.zeros((2 * HQ, 512), u32)
            vt_scr[0] = jnp.zeros((D, TQ), bf16)
            vt_scr[1] = jnp.zeros((D, TQ), bf16)

        def wait(*names):
            for name in names:
                copies[name].wait()

        def vfirst():
            qkv(1, 0, 5)
            wait('v')
            qkv(0, 10, 15)

        def run(item):
            if item is not None:
                item[0](*item[1:])

        if first:
            for name in ('xa', 'k', 'q', 'v', 'wo', 'b1', 'b2', 'w1', 'xb', 'w2', 'xc'):
                copies[name].start()
            zero_hist()
            wait('xa')
            ln1(0)
            ln1(1)
            wait('k')
            qkv(0, 5, 10)
            qkv(1, 5, 10)
            wait('q')
            qkv(0, 0, 5)
            att_a(0, 0)
            y0 = [(vfirst,), (qkv, 1, 10, 12), (qkv, 1, 12, 15)] + [None] * 5
            y1 = [None] * NG
            tail = [(wait, 'wo', 'w1', 'b1', 'b2'), (biases,), (oproj, 0), (oproj, 1), (ffn1, 0, 0, 4),
                    (ffn1, 0, 4, 8), (ffn1, 0, 8, 12)]
        elif not redo:
            shift_hist()
            biases()
            ln1_load()
            qkv(0, 5, 10)
            ln1(1)
            qkv(0, 10, 15)
            qkv(0, 0, 5)
            att_a(0, 0)
            y0 = [(qkv, 1, 5, 7), (qkv, 1, 7, 10), (qkv, 1, 10, 12), (qkv, 1, 12, 15), (qkv, 1, 0, 2),
                  (qkv, 1, 2, 5), None, None]
            y1 = [None, (oproj, 0), None, (ffn1, 0, 0, 4), None, (ffn1, 0, 4, 8), None, (ffn1, 0, 8, 12)]
            tail = [(ffn2, 0, 0, 4), (oproj, 1), (ffn2, 0, 4, 8), (ffn2, 0, 8, 12), (fin, 0)]
        else:
            biases()
            att_a(0, 0)
            y0 = [None] * NG
            y1 = [None, (oproj, 0), None, (ffn1, 0, 0, 4), None, (ffn1, 0, 4, 8), None, (ffn1, 0, 8, 12)]
            tail = [(ffn2, 0, 0, 4), (oproj, 1), (ffn2, 0, 4, 8), (ffn2, 0, 8, 12), (fin, 0)]
        for g in range(NG):
            if g + 1 < NG:
                att_a(0, g + 1)
            else:
                att_a(1, 0)
            att_b(0, g)
            run(y0[g])
            att_c(0, g)
        for g in range(NG):
            if g + 1 < NG:
                att_a(1, g + 1)
            att_b(1, g)
            run(y1[g])
            att_c(1, g)
        for item in tail:
            run(item)
        if first:
            ffn1(1, 0, 4)
            ffn1(1, 4, 8)
            wait('xb', 'w2')
            ffn2(0, 0, 4)
            ffn1(1, 8, 12)
            ln1_next()
            ffn2(0, 4, 8)
            ffn2(0, 8, 12)
            fin(0)
            ffn2(1, 0, 4)
        else:
            ffn1(1, 0, 4)
            if not redo:
                ln1_next()
            ffn1(1, 4, 8)
            ffn2(1, 0, 4)
            ffn1(1, 8, 12)
        ffn2(1, 4, 8)
        ffn2(1, 8, 12)
        fin(1)
        if not redo:
            fin_ok = jnp.where((st8['fin', 0] + st8['fin', 1]) == 0.0, 0.0, 1.0)
            bad_ref[0] = jnp.maximum(jnp.max(st8['bad']), jnp.max(fin_ok))

    @pl.when(s == 0)
    def _():
        body('first')

    @pl.when(s == 1)
    def _():
        copies['xc'].wait()

    @pl.when(s > 0)
    def _():
        body('fast')

    @pl.when(bad_ref[0] > 0.0)
    def _():
        body('redo')


@jax.jit
def pallas_sequential_preLN__sliding_block__dense_activation_gelu__prompt_kernel(
    A_x, A_wqkv, A_wo, B_x, B_w1, B_b1, B_w2, B_b2):
    x = A_x.reshape(S, D)
    hbm = pl.BlockSpec(memory_space=pl.ANY)
    out = pl.pallas_call(
        kernel,
        grid=(S // T,),
        in_specs=[hbm] * 7,
        out_specs=pl.BlockSpec((T, D), lambda i: (i, 0)),
        out_shape=jax.ShapeDtypeStruct((S, D), bf16),
        scratch_shapes=[
            pltpu.VMEM((S, D), bf16),
            pltpu.VMEM((D, 3 * D), bf16),
            pltpu.VMEM((D, D), bf16),
            pltpu.VMEM((D, F), bf16),
            pltpu.VMEM((F,), bf16),
            pltpu.VMEM((F, D), bf16),
            pltpu.VMEM((D,), bf16),
            pltpu.SemaphoreType.DMA((11,)),
            pltpu.SMEM((1,), f32),
            pltpu.VMEM((NTILES * HQ, D), u32),
            pltpu.VMEM((NTILES * HQ, 512), u32),
            pltpu.VMEM((NTILES, D, TQ), bf16),
            pltpu.VMEM((NQ * HQ, D), u32),
            pltpu.VMEM((NQ * HQ, 512), u32),
            pltpu.VMEM((D, T), f32),
            pltpu.VMEM((TQ, D), bf16),
            pltpu.VMEM((HQ, D), u32),
        ],
        compiler_params=pltpu.CompilerParams(
            dimension_semantics=("arbitrary",),
            vmem_limit_bytes=100 * 1024 * 1024,
        ),
    )(x, A_wqkv, A_wo, B_w1, B_b1, B_w2, B_b2)
    return out.reshape(1, S, D)
```

```python
import math
import jax
import jax.numpy as jnp
from jax import lax
import jax.experimental.pallas as pl
import jax.experimental.pallas.tpu as pltpu

S, D, H, DH, W, F = 2048, 640, 32, 20, 256, 1536
TQ = 128
HQ = TQ // 2
NQ = 2
T = NQ * TQ
GH = 4
NG = H // GH
QN = TQ // GH
QW = QN // 2
NTILES = NQ + 2
EPS = 1e-5
QSCALE = (DH ** -0.5) * math.log2(math.e)
NEG = -1e9
LMAX = 2.0 ** 30
NT = (((1,), (1,)), ((), ()))
f32 = jnp.float32
bf16 = jnp.bfloat16
u32 = jnp.uint32
ONES2 = 0x3F803F80
FC = ((0, 4), (4, 8), (8, 12))


def _ln(x):
    m = jnp.mean(x, axis=-1, keepdims=True)
    xc = x - m
    v = jnp.mean(xc * xc, axis=-1, keepdims=True)
    return xc * lax.rsqrt(v + EPS)


def _gelu(x):
    c = math.sqrt(2.0 / math.pi)
    return 0.5 * x * (1.0 + jnp.tanh(c * (x + 0.044715 * (x * x * x))))


def _pack_halves(x):
    r = x.shape[0] // 2
    return pltpu.bitcast(pltpu.pack_elementwise([x[:r], x[r:]], packed_dtype=bf16), u32)


def _pack16(x):
    n = x.shape[0] // 16
    a = jnp.concatenate([x[16 * k:16 * k + 8] for k in range(n)], axis=0)
    b = jnp.concatenate([x[16 * k + 8:16 * k + 16] for k in range(n)], axis=0)
    return pltpu.bitcast(pltpu.pack_elementwise([a, b], packed_dtype=bf16), u32)


def _group_tile(g):
    c0 = g * GH * DH
    t = c0 // 128
    if (c0 + GH * DH - 1) // 128 == t:
        return False, t, c0 - t * 128
    t = (c0 - 64) // 128
    assert c0 + GH * DH <= t * 128 + 192
    return True, t, c0 - (t * 128 + 64)


def _rows(j, unit, off, n):
    if isinstance(j, int):
        return slice(j * unit + off, j * unit + off + n)
    return pl.ds(pl.multiple_of(j * unit + off, 16), n)


def _kernel(x_hbm, wqkv_hbm, wo_hbm, w1_hbm, b1_hbm, w2_hbm, b2_hbm, o_ref,
            x_ref, wqkv_ref, wo_ref, w1_ref, b1_ref, w2_ref, b2_ref, sems, bad_ref,
            k_scr, ks_scr, vt_scr, q_scr, qs_scr, ot_scr, xt_scr, xs_scr):
    s = pl.program_id(0)

    def slab(i, sem):
        return pltpu.make_async_copy(wqkv_hbm.at[:, i * D:(i + 1) * D], wqkv_ref.at[:, i * D:(i + 1) * D],
                                     sems.at[sem])

    def xrows(r0, r1, sem):
        return pltpu.make_async_copy(x_hbm.at[r0:r1, :], x_ref.at[r0:r1, :], sems.at[sem])

    copies = {
        'q': slab(0, 0), 'k': slab(1, 1), 'v': slab(2, 2),
        'wo': pltpu.make_async_copy(wo_hbm, wo_ref, sems.at[3]),
        'w1': pltpu.make_async_copy(w1_hbm, w1_ref, sems.at[4]),
        'w2': pltpu.make_async_copy(w2_hbm, w2_ref, sems.at[5]),
        'b1': pltpu.make_async_copy(b1_hbm, b1_ref, sems.at[6]),
        'b2': pltpu.make_async_copy(b2_hbm, b2_ref, sems.at[7]),
        'xa': xrows(0, T, 8), 'xb': xrows(T, T + TQ, 9), 'xc': xrows(T + TQ, S, 10),
    }

    def body(mode, zdyn=None):
        first, redo = mode == 'first', mode == 'redo'
        row0 = 0 if first else pl.multiple_of(s * T, T)

        ki = lax.broadcasted_iota(jnp.int32, (QN, TQ), 0)
        qi = lax.broadcasted_iota(jnp.int32, (QN, TQ), 1) & (QN - 1)
        tri = ki > qi
        if not first:
            r2 = lax.broadcasted_iota(jnp.int32, (HQ, TQ), 0)
            r2 = r2 + (r2 & -8)
            l2 = lax.broadcasted_iota(jnp.int32, (HQ, TQ), 1)
            mus, mls = [], []
            for a in range(GH):
                q2 = l2 ^ (QN * a)
                mu = jnp.where(r2 > q2, 0xFFFF, 0) | jnp.where(r2 + 8 > q2, -65536, 0)
                mu = pltpu.bitcast(mu, u32)
                mus.append(mu)
                mls.append(~mu)
        if redo:
            b_old = jnp.where(s * NQ + zdyn >= 2, 0.0, NEG).astype(f32)
            b_mid = jnp.where(s * NQ + zdyn >= 1, 0.0, NEG).astype(f32)

        def butterfly(ts):
            lane = lax.broadcasted_iota(jnp.int32, ts[0].shape, 1)
            odd = (lane & QN) != 0
            us = [jnp.where(odd, ts[c ^ 1], ts[c]) for c in range(GH)]
            hi = (lane & (2 * QN)) != 0
            return [jnp.where(hi, us[a ^ 2], us[a]) for a in range(GH)]

        st8 = {'bad': jnp.zeros((1, TQ), f32), 'fin': jnp.zeros((1, D), f32)}

        def key(z):
            return z if isinstance(z, int) else 'dyn'

        def xblk(z):
            return x_ref[pl.ds(pl.multiple_of(row0 + z * TQ, TQ), TQ), :]

        def ln1_vals(xb):
            xu = pltpu.bitcast(xb, u32)
            xe = pltpu.unpack_elementwise(xu, index=0, packed_dtype=bf16, unpacked_dtype=f32)
            xo = pltpu.unpack_elementwise(xu, index=1, packed_dtype=bf16, unpacked_dtype=f32)
            xn = _ln(jnp.concatenate([xe, xo], axis=0))
            nat = pltpu.bitcast(_pack_halves(xn), bf16).astype(f32)
            return xn.astype(bf16), _pack16(nat)

        def ln1(z):
            xt, xs = ln1_vals(xblk(z))
            st8['xt', z] = xt
            st8['xs', z] = pltpu.bitcast(xs, bf16)

        def ln1_load():
            st8['xt', 0] = xt_scr[...]
            st8['xs', 0] = pltpu.bitcast(xs_scr[...], bf16)

        def ln1_next():
            nxt = T if first else pl.multiple_of(jnp.minimum(row0 + T, S - TQ), TQ)
            xt, xs = ln1_vals(x_ref[pl.ds(nxt, TQ), :])
            xt_scr[...] = xt
            xs_scr[...] = xs

        def qkv(z, t0, t1):
            xn = st8['xs' if t0 >= 10 else 'xt', z]
            r = jnp.dot(xn, wqkv_ref[:, t0 * 128:t1 * 128], preferred_element_type=f32)
            for t in range(t0, t1):
                rt = r[:, (t - t0) * 128:(t - t0 + 1) * 128]
                if t < 5:
                    q_scr[z * HQ:(z + 1) * HQ, t * 128:(t + 1) * 128] = _pack_halves(rt * QSCALE)
                elif t < 10:
                    k_scr[(z + 2) * HQ:(z + 3) * HQ, (t - 5) * 128:(t - 4) * 128] = _pack_halves(rt)
                else:
                    vt_scr[z + 2, (t - 10) * 128:(t - 9) * 128, :] = rt.T.astype(bf16)
            if t1 == 5:
                qs_scr[z * HQ:(z + 1) * HQ, :] = q_scr[z * HQ:(z + 1) * HQ, 64:576]
            if t1 == 10:
                ks_scr[(z + 2) * HQ:(z + 3) * HQ, :] = k_scr[(z + 2) * HQ:(z + 3) * HQ, 64:576]

        def ntiles(j):
            return min(3, j + 1) if first else 3

        def stage_a1(j, g, c):
            nt = ntiles(j)
            sh, t, lo = _group_tile(g)
            qr, kr = (qs_scr, ks_scr) if sh else (q_scr, k_scr)
            lt = slice(t * 128, (t + 1) * 128)
            lane = lax.broadcasted_iota(jnp.int32, (QW, 128), 1)
            qc = qr[_rows(j, HQ, c * QW, QW), lt]
            qs = []
            for lam in range(GH):
                l0 = lo + (lam ^ c) * DH
                lm = pltpu.bitcast(jnp.where((lane >= l0) & (lane < l0 + DH), -1, 0), u32)
                qs.append(qc & lm)
            qm = pltpu.bitcast(jnp.concatenate(qs, axis=0), bf16)
            d0 = 2 * HQ + c * QW
            w0 = c * QW if nt == 3 else (3 - nt) * HQ
            kw = kr[_rows(j, HQ, d0, QW), lt]
            if d0 > w0:
                kw = jnp.concatenate([kw, kr[_rows(j, HQ, w0, d0 - w0), lt]], axis=0)
            st = lax.dot_general(pltpu.bitcast(kw, bf16), qm, NT, preferred_element_type=f32)
            n = st.shape[0]
            parts = [st[n - QN * c:n]] if c > 0 else []
            if nt == 3:
                old = st[QN:TQ - QN * c + QN]
                if redo:
                    old = old + b_old
                parts.append(jnp.where(tri, old[0:QN], st[0:QN]))
                if c < GH - 1:
                    parts.append(old[QN:])
            else:
                parts.append(jnp.where(tri, NEG, st[0:QN]))
            sm = jnp.concatenate(parts, axis=0) if len(parts) > 1 else parts[0]
            s1 = st[n - QN * c - TQ:n - QN * c] if nt > 1 else None
            if redo:
                s1 = s1 + b_mid
                m = jnp.max(jnp.maximum(sm, s1), axis=0, keepdims=True)
            else:
                m = jnp.max(jnp.where(tri, NEG, st[0:QN]), axis=0, keepdims=True)
            return sm, s1, m

        def stage_b1(sm, s1, m):
            pm = jnp.exp2(sm - m)
            if pm.shape[0] < TQ:
                pm = jnp.concatenate([pm, jnp.zeros((TQ - pm.shape[0], TQ), f32)], axis=0)
            if s1 is None:
                return _pack16(pm), None
            return _pack16(pm), _pack16(jnp.exp2(s1 - m))

        def stage_c1(j, h, pmu, p1u):
            nt = ntiles(j)
            c0 = h * DH
            if nt == 3:
                parts = [pmu & mus[h % GH], p1u, pmu & mls[h % GH]]
            elif nt == 2:
                parts = [p1u, pmu]
            else:
                parts = [pmu]
            pb = jnp.concatenate([pltpu.bitcast(p, bf16) for p in parts], axis=0)
            r0 = (c0 // 16) * 16
            off = c0 - r0
            vt = jnp.concatenate([vt_scr[j + t, r0:r0 + 32, :] for t in range(3 - nt, 3)], axis=1)
            vu = pltpu.bitcast(vt, u32)
            wrow = lax.broadcasted_iota(jnp.int32, (8, nt * TQ), 0)
            if off < 12:
                lrow = 30
                vu = jnp.concatenate([vu[0:8], jnp.where(wrow == 7, jnp.uint32(ONES2), vu[8:16])], axis=0)
            else:
                lrow = 0
                vu = jnp.concatenate([jnp.where(wrow == 0, jnp.uint32(ONES2), vu[0:8]), vu[8:16]], axis=0)
            ot = jnp.dot(pltpu.bitcast(vu, bf16), pb, preferred_element_type=f32)
            l = ot[lrow:lrow + 1, :]
            if not redo:
                st8['bad'] = jnp.where(l <= LMAX, st8['bad'], 1.0)
            ot = ot * (1.0 / l)
            ot_scr[j, c0:c0 + DH, :] = ot[off:off + DH, :]

        def att_a(z, g):
            st8['s', key(z), g] = [stage_a1(z, g, c) for c in range(GH)]

        def att_b(z, g):
            st8['p', key(z), g] = [stage_b1(*a) for a in st8.pop(('s', key(z), g))]

        def att_c(z, g):
            rs = st8.pop(('p', key(z), g))
            pms = butterfly([r[0] for r in rs])
            p1s = butterfly([r[1] for r in rs]) if rs[0][1] is not None else [None] * GH
            for a in range(GH):
                stage_c1(z, g * GH + a, pms[a], p1s[a])

        def otr(z):
            o = ot_scr[z].T
            if not redo:
                st8['fin'] = st8['fin'] + jnp.sum(o - o, axis=0, keepdims=True)
            hid = lax.broadcasted_iota(jnp.int32, (QN, D), 1) // DH
            bs = [o[QN * i:QN * (i + 1)] for i in range(GH)]
            odd = (hid & 1) != 0
            us = [jnp.where(odd, bs[i ^ 1], bs[i]) for i in range(GH)]
            hi = (hid & 2) != 0
            st8['o', key(z)] = jnp.concatenate([jnp.where(hi, us[i ^ 2], us[i]) for i in range(GH)],
                                               axis=0).astype(bf16)

        def oproj(z):
            if ('o', key(z)) not in st8:
                otr(z)
            h1 = xblk(z).astype(f32) + jnp.dot(st8.pop(('o', key(z))), wo_ref[...],
                                               preferred_element_type=f32)
            st8['h', key(z)] = h1
            st8['hn', key(z)] = _ln(h1).astype(bf16)

        def biases():
            st8['b1'] = b1_ref[...].astype(f32).reshape(1, F)
            st8['b2'] = b2_ref[...].astype(f32).reshape(1, D)

        def ffn1(z, c0, c1):
            u = jnp.dot(st8['hn', key(z)], w1_ref[:, c0 * 128:c1 * 128], preferred_element_type=f32)
            st8['u', key(z), c0] = _gelu(u + st8['b1'][:, c0 * 128:c1 * 128]).astype(bf16)

        def ffn2(z, c0, c1):
            y = jnp.dot(st8.pop(('u', key(z), c0)), w2_ref[c0 * 128:c1 * 128, :], preferred_element_type=f32)
            st8['h', key(z)] = st8['h', key(z)] + y

        def fin(z):
            o_ref[_rows(z, TQ, 0, TQ), :] = (st8['h', key(z)] + st8['b2']).astype(o_ref.dtype)

        def shift_hist():
            k_scr[0:2 * HQ, :] = k_scr[NQ * HQ:(NQ + 2) * HQ, :]
            ks_scr[0:2 * HQ, :] = ks_scr[NQ * HQ:(NQ + 2) * HQ, :]
            vt_scr[0] = vt_scr[NQ]
            vt_scr[1] = vt_scr[NQ + 1]

        def zero_hist():
            k_scr[0:2 * HQ, :] = jnp.zeros((2 * HQ, D), u32)
            ks_scr[0:2 * HQ, :] = jnp.zeros((2 * HQ, 512), u32)
            vt_scr[0] = jnp.zeros((D, TQ), bf16)
            vt_scr[1] = jnp.zeros((D, TQ), bf16)

        def wait(*names):
            for name in names:
                copies[name].wait()

        def run(items):
            for item in items:
                item[0](*item[1:])

        if redo:
            z = zdyn
            biases()
            att_a(z, 0)
            for g in range(NG):
                if g + 1 < NG:
                    att_a(z, g + 1)
                att_b(z, g)
                att_c(z, g)
            oproj(z)
            for c in FC:
                ffn1(z, *c)
            for c in FC:
                ffn2(z, *c)
            fin(z)
            return

        slots = [[[] for _ in range(NG)] for _ in range(NQ)]
        if first:
            for name in ('xa', 'k', 'q', 'v', 'wo', 'b1', 'b2', 'w1', 'xb', 'w2', 'xc'):
                copies[name].start()
            zero_hist()
            wait('xa')
            ln1(0)
            ln1(1)
            wait('k')
            qkv(0, 5, 10)
            qkv(1, 5, 10)
            wait('q')
            qkv(0, 0, 5)
            slots[0][0] = [(qkv, 1, 0, 5), (wait, 'v'), (qkv, 0, 10, 15)]
            slots[0][1] = [(qkv, 1, 10, 12)]
            slots[0][2] = [(qkv, 1, 12, 15)]
            slots[1][1] = [(otr, 0)]
            tail = [(wait, 'wo', 'w1', 'b1', 'b2'), (biases,), (oproj, 0), (oproj, 1)]
            tail += [(ffn1, 0, *c) for c in FC]
            tail += [(ffn1, 1, 0, 4), (ffn1, 1, 4, 8), (wait, 'xb', 'w2'), (ffn2, 0, 0, 4), (ffn1, 1, 8, 12),
                     (ln1_next,), (ffn2, 0, 4, 8), (ffn2, 0, 8, 12), (fin, 0), (ffn2, 1, 0, 4)]
        else:
            biases()
            shift_hist()
            ln1_load()
            qkv(0, 5, 10)
            ln1(1)
            qkv(0, 0, 5)
            qkv(0, 10, 15)
            for i, c in enumerate(((5, 7), (7, 10), (10, 12), (12, 15), (0, 2), (2, 5))):
                slots[0][i] = [(qkv, 1, *c)]
            slots[1][1] = [(oproj, 0)]
            for i, c in enumerate(FC):
                slots[1][3 + 2 * i] = [(ffn1, 0, *c)]
            tail = [(ffn2, 0, 0, 4), (oproj, 1), (ffn2, 0, 4, 8), (ffn2, 0, 8, 12), (fin, 0),
                    (ffn1, 1, 0, 4), (ln1_next,), (ffn1, 1, 4, 8), (ffn2, 1, 0, 4), (ffn1, 1, 8, 12)]
        att_a(0, 0)
        for z in range(NQ):
            for g in range(NG):
                if g + 1 < NG:
                    att_a(z, g + 1)
                elif z + 1 < NQ:
                    att_a(z + 1, 0)
                att_b(z, g)
                run(slots[z][g])
                att_c(z, g)
        run(tail + [(ffn2, 1, 4, 8), (ffn2, 1, 8, 12), (fin, 1)])
        not_finite = jnp.where(st8['fin'] == 0.0, 0.0, 1.0)
        bad_ref[0] = jnp.maximum(jnp.max(st8['bad']), jnp.max(not_finite))

    @pl.when(s == 0)
    def _():
        body('first')

    @pl.when(s == 1)
    def _():
        copies['xc'].wait()

    @pl.when(s > 0)
    def _():
        body('fast')

    @pl.when(bad_ref[0] > 0.0)
    def _():
        def redo_tile(z, carry):
            body('redo', z)
            return carry

        lax.fori_loop(0, NQ, redo_tile, 0)


@jax.jit
def pallas_sequential_preLN__sliding_block__dense_activation_gelu__prompt_kernel(
    A_x: jax.Array,
    A_wqkv: jax.Array,
    A_wo: jax.Array,
    B_x: jax.Array,
    B_w1: jax.Array,
    B_b1: jax.Array,
    B_w2: jax.Array,
    B_b2: jax.Array,
):
    del B_x
    hbm = pl.BlockSpec(memory_space=pl.ANY)
    out = pl.pallas_call(
        _kernel,
        grid=(S // T,),
        in_specs=[hbm] * 7,
        out_specs=pl.BlockSpec((T, D), lambda i: (i, 0)),
        out_shape=jax.ShapeDtypeStruct((S, D), bf16),
        scratch_shapes=[
            pltpu.VMEM((S, D), bf16),
            pltpu.VMEM((D, 3 * D), bf16),
            pltpu.VMEM((D, D), bf16),
            pltpu.VMEM((D, F), bf16),
            pltpu.VMEM((F,), bf16),
            pltpu.VMEM((F, D), bf16),
            pltpu.VMEM((D,), bf16),
            pltpu.SemaphoreType.DMA((11,)),
            pltpu.SMEM((1,), f32),
            pltpu.VMEM((NTILES * HQ, D), u32),
            pltpu.VMEM((NTILES * HQ, 512), u32),
            pltpu.VMEM((NTILES, D, TQ), bf16),
            pltpu.VMEM((NQ * HQ, D), u32),
            pltpu.VMEM((NQ * HQ, 512), u32),
            pltpu.VMEM((NQ, D, TQ), f32),
            pltpu.VMEM((TQ, D), bf16),
            pltpu.VMEM((HQ, D), u32),
        ],
        compiler_params=pltpu.CompilerParams(
            dimension_semantics=("arbitrary",),
            vmem_limit_bytes=64 * 1024 * 1024,
        ),
    )(A_x.reshape(S, D), A_wqkv, A_wo, B_w1, B_b1, B_w2, B_b2)
    return out.reshape(1, S, D)
```

```python
import math
import jax
import jax.numpy as jnp
from jax import lax
import jax.experimental.pallas as pl
import jax.experimental.pallas.tpu as pltpu

S, D, H, DH, W, F = 2048, 640, 32, 20, 256, 1536
TQ = 128
HQ = TQ // 2
NQ = 2
T = NQ * TQ
GH = 4
NG = H // GH
QN = TQ // GH
QW = QN // 2
NTILES = NQ + 2
EPS = 1e-5
QSCALE = (DH ** -0.5) * math.log2(math.e)
NEG = -1e9
LMAX = 2.0 ** 30
PROUND = math.log2(1.0 + 3.0 * 2.0 ** -10)
NT = (((1,), (1,)), ((), ()))
f32 = jnp.float32
bf16 = jnp.bfloat16
u32 = jnp.uint32
ONES2 = 0x3F803F80
FC = ((0, 4), (4, 8), (8, 12))


def _ln(x):
    m = jnp.mean(x, axis=-1, keepdims=True)
    xc = x - m
    v = jnp.mean(xc * xc, axis=-1, keepdims=True)
    return xc * lax.rsqrt(v + EPS)


def _gelu(x):
    c = math.sqrt(2.0 / math.pi)
    return 0.5 * x * (1.0 + jnp.tanh(c * (x + 0.044715 * (x * x * x))))


def _pack2(a, b, rnd):
    ua = pltpu.bitcast(a, u32)
    ub = pltpu.bitcast(b, u32)
    if rnd:
        ua = ua + jnp.uint32(0x8000)
        ub = ub + jnp.uint32(0x8000)
    return (ua >> 16) | (ub & jnp.uint32(0xFFFF0000))


def _pack_halves(x):
    r = x.shape[0] // 2
    return _pack2(x[:r], x[r:], True)


def _pack16(x):
    n = x.shape[0] // 16
    a = jnp.concatenate([x[16 * k:16 * k + 8] for k in range(n)], axis=0)
    b = jnp.concatenate([x[16 * k + 8:16 * k + 16] for k in range(n)], axis=0)
    return _pack2(a, b, False)


def _group_tile(g):
    c0 = g * GH * DH
    t = c0 // 128
    if (c0 + GH * DH - 1) // 128 == t:
        return False, t, c0 - t * 128
    t = (c0 - 64) // 128
    assert c0 + GH * DH <= t * 128 + 192
    return True, t, c0 - (t * 128 + 64)


def _rows(j, unit, off, n):
    if isinstance(j, int):
        return slice(j * unit + off, j * unit + off + n)
    return pl.ds(pl.multiple_of(j * unit + off, 16), n)


def _kernel(x_hbm, wqkv_hbm, wo_hbm, w1_hbm, b1_hbm, w2_hbm, b2_hbm, o_ref,
            x_ref, wqkv_ref, wo_ref, w1_ref, b1_ref, w2_ref, b2_ref, sems, bad_ref,
            k_scr, ks_scr, vt_scr, q_scr, qs_scr, ot_scr, xt_scr, xs_scr):
    s = pl.program_id(0)

    def slab(i, sem):
        return pltpu.make_async_copy(wqkv_hbm.at[:, i * D:(i + 1) * D], wqkv_ref.at[:, i * D:(i + 1) * D],
                                     sems.at[sem])

    def xrows(r0, r1, sem):
        return pltpu.make_async_copy(x_hbm.at[r0:r1, :], x_ref.at[r0:r1, :], sems.at[sem])

    copies = {
        'q': slab(0, 0), 'k': slab(1, 1), 'v': slab(2, 2),
        'wo': pltpu.make_async_copy(wo_hbm, wo_ref, sems.at[3]),
        'w1': pltpu.make_async_copy(w1_hbm, w1_ref, sems.at[4]),
        'w2': pltpu.make_async_copy(w2_hbm, w2_ref, sems.at[5]),
        'b1': pltpu.make_async_copy(b1_hbm, b1_ref, sems.at[6]),
        'b2': pltpu.make_async_copy(b2_hbm, b2_ref, sems.at[7]),
        'xa': xrows(0, T, 8), 'xb': xrows(T, T + TQ, 9), 'xc': xrows(T + TQ, S, 10),
    }

    def body(mode, zdyn=None):
        first, redo = mode == 'first', mode == 'redo'
        row0 = 0 if first else s * T

        ki = lax.broadcasted_iota(jnp.int32, (QN, TQ), 0)
        qi = lax.broadcasted_iota(jnp.int32, (QN, TQ), 1) & (QN - 1)
        tri = ki > qi
        if not first:
            r2 = lax.broadcasted_iota(jnp.int32, (HQ, TQ), 0)
            r2 = r2 + (r2 & -8)
            l2 = lax.broadcasted_iota(jnp.int32, (HQ, TQ), 1)
            mus, mls = [], []
            for a in range(GH):
                q2 = l2 ^ (QN * a)
                mu = jnp.where(r2 > q2, 0xFFFF, 0) | jnp.where(r2 + 8 > q2, -65536, 0)
                mu = pltpu.bitcast(mu, u32)
                mus.append(mu)
                mls.append(~mu)
        if redo:
            b_old = jnp.where(s * NQ + zdyn >= 2, 0.0, NEG).astype(f32)
            b_mid = jnp.where(s * NQ + zdyn >= 1, 0.0, NEG).astype(f32)

        def butterfly(ts):
            lane = lax.broadcasted_iota(jnp.int32, ts[0].shape, 1)
            odd = (lane & QN) != 0
            us = [jnp.where(odd, ts[c ^ 1], ts[c]) for c in range(GH)]
            hi = (lane & (2 * QN)) != 0
            return [jnp.where(hi, us[a ^ 2], us[a]) for a in range(GH)]

        st8 = {'bad': jnp.zeros((1, TQ), f32), 'fin': jnp.zeros((1, D), f32)}

        def key(z):
            return z if isinstance(z, int) else 'dyn'

        def xtile(r):
            return x_ref[r:r + TQ, :] if isinstance(r, int) else x_ref[pl.ds(pl.multiple_of(r, TQ), TQ), :]

        def xblk(z):
            return xtile(row0 + z * TQ)

        def ln1_vals(xb):
            xu = pltpu.bitcast(xb, u32)
            xe = pltpu.bitcast(xu << 16, f32)
            xo = pltpu.bitcast(xu & jnp.uint32(0xFFFF0000), f32)
            xn = _ln(jnp.concatenate([xe, xo], axis=0))
            nat = pltpu.bitcast(_pack_halves(xn), bf16).astype(f32)
            return xn.astype(bf16), _pack16(nat)

        def ln1(z):
            xt, xs = ln1_vals(xblk(z))
            st8['xt', z] = xt
            st8['xs', z] = pltpu.bitcast(xs, bf16)

        def ln1_load():
            st8['xt', 0] = xt_scr[...]
            st8['xs', 0] = pltpu.bitcast(xs_scr[...], bf16)

        def ln1_next():
            xt, xs = ln1_vals(xtile(T if first else jnp.minimum(row0 + T, S - TQ)))
            xt_scr[...] = xt
            xs_scr[...] = xs

        def qkv(z, t0, t1):
            xn = st8['xs' if t0 >= 10 else 'xt', z]
            r = jnp.dot(xn, wqkv_ref[:, t0 * 128:t1 * 128], preferred_element_type=f32)
            for t in range(t0, t1):
                rt = r[:, (t - t0) * 128:(t - t0 + 1) * 128]
                if t < 5:
                    q_scr[z * HQ:(z + 1) * HQ, t * 128:(t + 1) * 128] = _pack_halves(rt * QSCALE)
                elif t < 10:
                    k_scr[(z + 2) * HQ:(z + 3) * HQ, (t - 5) * 128:(t - 4) * 128] = _pack_halves(rt)
                else:
                    vt_scr[z + 2, (t - 10) * 128:(t - 9) * 128, :] = rt.T.astype(bf16)
            if t1 == 5:
                qs_scr[z * HQ:(z + 1) * HQ, :] = q_scr[z * HQ:(z + 1) * HQ, 64:576]
            if t1 == 10:
                ks_scr[(z + 2) * HQ:(z + 3) * HQ, :] = k_scr[(z + 2) * HQ:(z + 3) * HQ, 64:576]

        def ntiles(j):
            return min(3, j + 1) if first else 3

        def stage_a1(j, g, c):
            nt = ntiles(j)
            sh, t, lo = _group_tile(g)
            qr, kr = (qs_scr, ks_scr) if sh else (q_scr, k_scr)
            lt = slice(t * 128, (t + 1) * 128)
            lane = lax.broadcasted_iota(jnp.int32, (QW, 128), 1)
            qc = qr[_rows(j, HQ, c * QW, QW), lt]
            qs = []
            for lam in range(GH):
                l0 = lo + (lam ^ c) * DH
                lm = pltpu.bitcast(jnp.where((lane >= l0) & (lane < l0 + DH), -1, 0), u32)
                qs.append(qc & lm)
            qm = pltpu.bitcast(jnp.concatenate(qs, axis=0), bf16)
            d0 = 2 * HQ + c * QW
            w0 = c * QW if nt == 3 else (3 - nt) * HQ
            kw = kr[_rows(j, HQ, d0, QW), lt]
            if d0 > w0:
                kw = jnp.concatenate([kw, kr[_rows(j, HQ, w0, d0 - w0), lt]], axis=0)
            st = lax.dot_general(pltpu.bitcast(kw, bf16), qm, NT, preferred_element_type=f32)
            n = st.shape[0]
            parts = [st[n - QN * c:n]] if c > 0 else []
            if nt == 3:
                old = st[QN:TQ - QN * c + QN]
                if redo:
                    old = old + b_old
                parts.append(jnp.where(tri, old[0:QN], st[0:QN]))
                if c < GH - 1:
                    parts.append(old[QN:])
            else:
                parts.append(jnp.where(tri, NEG, st[0:QN]))
            sm = jnp.concatenate(parts, axis=0) if len(parts) > 1 else parts[0]
            s1 = st[n - QN * c - TQ:n - QN * c] if nt > 1 else None
            if redo:
                s1 = s1 + b_mid
                m = jnp.max(jnp.maximum(sm, s1), axis=0, keepdims=True)
            else:
                m = jnp.max(jnp.where(tri, NEG, st[0:QN]), axis=0, keepdims=True)
            return sm, s1, m

        def stage_b1(sm, s1, m):
            m = m - PROUND
            pm = jnp.exp2(sm - m)
            if pm.shape[0] < TQ:
                pm = jnp.concatenate([pm, jnp.zeros((TQ - pm.shape[0], TQ), f32)], axis=0)
            if s1 is None:
                return _pack16(pm), None
            return _pack16(pm), _pack16(jnp.exp2(s1 - m))

        def stage_c1(j, h, pmu, p1u):
            nt = ntiles(j)
            c0 = h * DH
            if nt == 3:
                parts = [pmu & mus[h % GH], p1u, pmu & mls[h % GH]]
            elif nt == 2:
                parts = [p1u, pmu]
            else:
                parts = [pmu]
            pb = jnp.concatenate([pltpu.bitcast(p, bf16) for p in parts], axis=0)
            r0 = (c0 // 16) * 16
            off = c0 - r0
            vt = jnp.concatenate([vt_scr[j + t, r0:r0 + 32, :] for t in range(3 - nt, 3)], axis=1)
            vu = pltpu.bitcast(vt, u32)
            wrow = lax.broadcasted_iota(jnp.int32, (8, nt * TQ), 0)
            if off < 12:
                lrow = 30
                vu = jnp.concatenate([vu[0:8], jnp.where(wrow == 7, jnp.uint32(ONES2), vu[8:16])], axis=0)
            else:
                lrow = 0
                vu = jnp.concatenate([jnp.where(wrow == 0, jnp.uint32(ONES2), vu[0:8]), vu[8:16]], axis=0)
            ot = jnp.dot(pltpu.bitcast(vu, bf16), pb, preferred_element_type=f32)
            l = ot[lrow:lrow + 1, :]
            if not redo:
                st8['bad'] = jnp.where(l <= LMAX, st8['bad'], 1.0)
            ot = ot * (1.0 / l)
            ot_scr[j, c0:c0 + DH, :] = ot[off:off + DH, :]

        def att_a(z, g):
            st8['s', key(z), g] = [stage_a1(z, g, c) for c in range(GH)]

        def att_b(z, g):
            st8['p', key(z), g] = [stage_b1(*a) for a in st8.pop(('s', key(z), g))]

        def att_c(z, g):
            rs = st8.pop(('p', key(z), g))
            pms = butterfly([r[0] for r in rs])
            p1s = butterfly([r[1] for r in rs]) if rs[0][1] is not None else [None] * GH
            for a in range(GH):
                stage_c1(z, g * GH + a, pms[a], p1s[a])

        def otr(z):
            o = ot_scr[z].T
            if not redo:
                st8['fin'] = st8['fin'] + jnp.sum(o - o, axis=0, keepdims=True)
            hid = lax.broadcasted_iota(jnp.int32, (QN, D), 1) // DH
            bs = [o[QN * i:QN * (i + 1)] for i in range(GH)]
            odd = (hid & 1) != 0
            us = [jnp.where(odd, bs[i ^ 1], bs[i]) for i in range(GH)]
            hi = (hid & 2) != 0
            st8['o', key(z)] = jnp.concatenate([jnp.where(hi, us[i ^ 2], us[i]) for i in range(GH)],
                                               axis=0).astype(bf16)

        def oproj(z):
            if ('o', key(z)) not in st8:
                otr(z)
            h1 = xblk(z).astype(f32) + jnp.dot(st8.pop(('o', key(z))), wo_ref[...],
                                               preferred_element_type=f32)
            st8['h', key(z)] = h1
            st8['hn', key(z)] = _ln(h1).astype(bf16)

        def biases():
            st8['b1'] = b1_ref[...].astype(f32).reshape(1, F)
            st8['b2'] = b2_ref[...].astype(f32).reshape(1, D)

        def ffn1(z, c0, c1):
            u = jnp.dot(st8['hn', key(z)], w1_ref[:, c0 * 128:c1 * 128], preferred_element_type=f32)
            st8['u', key(z), c0] = _gelu(u + st8['b1'][:, c0 * 128:c1 * 128]).astype(bf16)

        def ffn2(z, c0, c1):
            y = jnp.dot(st8.pop(('u', key(z), c0)), w2_ref[c0 * 128:c1 * 128, :], preferred_element_type=f32)
            st8['h', key(z)] = st8['h', key(z)] + y

        def fin(z):
            o_ref[_rows(z, TQ, 0, TQ), :] = (st8['h', key(z)] + st8['b2']).astype(o_ref.dtype)

        def shift_hist():
            k_scr[0:2 * HQ, :] = k_scr[NQ * HQ:(NQ + 2) * HQ, :]
            ks_scr[0:2 * HQ, :] = ks_scr[NQ * HQ:(NQ + 2) * HQ, :]
            vt_scr[0] = vt_scr[NQ]
            vt_scr[1] = vt_scr[NQ + 1]

        def zero_hist():
            k_scr[0:2 * HQ, :] = jnp.zeros((2 * HQ, D), u32)
            ks_scr[0:2 * HQ, :] = jnp.zeros((2 * HQ, 512), u32)
            vt_scr[0] = jnp.zeros((D, TQ), bf16)
            vt_scr[1] = jnp.zeros((D, TQ), bf16)

        def wait(*names):
            for name in names:
                copies[name].wait()

        def run(items):
            for item in items:
                item[0](*item[1:])

        if redo:
            z = zdyn
            biases()
            att_a(z, 0)
            for g in range(NG):
                if g + 1 < NG:
                    att_a(z, g + 1)
                att_b(z, g)
                att_c(z, g)
            oproj(z)
            for c in FC:
                ffn1(z, *c)
            for c in FC:
                ffn2(z, *c)
            fin(z)
            return

        slots = [[[] for _ in range(NG)] for _ in range(NQ)]
        if first:
            for name in ('xa', 'k', 'q', 'v', 'wo', 'b1', 'b2', 'w1', 'xb', 'w2', 'xc'):
                copies[name].start()
            zero_hist()
            wait('xa')
            ln1(0)
            ln1(1)
            wait('k')
            qkv(0, 5, 10)
            qkv(1, 5, 10)
            wait('q')
            qkv(0, 0, 5)
            slots[0][0] = [(qkv, 1, 0, 5), (wait, 'v'), (qkv, 0, 10, 15)]
            slots[0][3] = [(qkv, 1, 10, 12)]
            slots[0][5] = [(qkv, 1, 12, 15)]
            slots[1][1] = [(otr, 0)]
            tail = [(wait, 'wo', 'w1', 'b1', 'b2'), (biases,), (oproj, 0), (oproj, 1)]
            tail += [(ffn1, 0, *c) for c in FC]
            tail += [(ffn1, 1, 0, 4), (ffn1, 1, 4, 8), (wait, 'xb', 'w2'), (ffn2, 0, 0, 4), (ffn1, 1, 8, 12),
                     (ln1_next,), (ffn2, 0, 4, 8), (ffn2, 0, 8, 12), (fin, 0), (ffn2, 1, 0, 4)]
        else:
            biases()
            shift_hist()
            ln1_load()
            qkv(0, 5, 10)
            ln1(1)
            qkv(0, 0, 5)
            qkv(0, 10, 15)
            for i, c in enumerate(((5, 7), (7, 10), (10, 12), (12, 15), (0, 2), (2, 5))):
                slots[0][i] = [(qkv, 1, *c)]
            slots[1][1] = [(oproj, 0)]
            for i, c in enumerate(FC):
                slots[1][3 + 2 * i] = [(ffn1, 0, *c)]
            tail = [(ffn2, 0, 0, 4), (oproj, 1), (ffn2, 0, 4, 8), (ffn2, 0, 8, 12), (fin, 0),
                    (ffn1, 1, 0, 4), (ln1_next,), (ffn1, 1, 4, 8), (ffn2, 1, 0, 4), (ffn1, 1, 8, 12)]
        att_a(0, 0)
        for z in range(NQ):
            for g in range(NG):
                if g + 1 < NG:
                    att_a(z, g + 1)
                elif z + 1 < NQ:
                    att_a(z + 1, 0)
                att_b(z, g)
                run(slots[z][g])
                att_c(z, g)
        run(tail + [(ffn2, 1, 4, 8), (ffn2, 1, 8, 12), (fin, 1)])
        not_finite = jnp.where(st8['fin'] == 0.0, 0.0, 1.0)
        bad_ref[0] = jnp.maximum(jnp.max(st8['bad']), jnp.max(not_finite))

    bad_ref[0] = jnp.float32(0.0)

    @pl.when(s == 0)
    def _():
        body('first')

    @pl.when(s == 1)
    def _():
        copies['xc'].wait()

    @pl.when(s > 0)
    def _():
        body('fast')

    @pl.when(bad_ref[0] > 0.0)
    def _():
        def redo_tile(z, carry):
            body('redo', z)
            return carry

        lax.fori_loop(0, NQ, redo_tile, 0)


@jax.jit
def pallas_sequential_preLN__sliding_block__dense_activation_gelu__prompt_kernel(
    A_x: jax.Array,
    A_wqkv: jax.Array,
    A_wo: jax.Array,
    B_x: jax.Array,
    B_w1: jax.Array,
    B_b1: jax.Array,
    B_w2: jax.Array,
    B_b2: jax.Array,
):
    del B_x
    hbm = pl.BlockSpec(memory_space=pl.ANY)
    out = pl.pallas_call(
        _kernel,
        grid=(S // T,),
        in_specs=[hbm] * 7,
        out_specs=pl.BlockSpec((T, D), lambda i: (i, 0)),
        out_shape=jax.ShapeDtypeStruct((S, D), bf16),
        scratch_shapes=[
            pltpu.VMEM((S, D), bf16),
            pltpu.VMEM((D, 3 * D), bf16),
            pltpu.VMEM((D, D), bf16),
            pltpu.VMEM((D, F), bf16),
            pltpu.VMEM((F,), bf16),
            pltpu.VMEM((F, D), bf16),
            pltpu.VMEM((D,), bf16),
            pltpu.SemaphoreType.DMA((11,)),
            pltpu.SMEM((1,), f32),
            pltpu.VMEM((NTILES * HQ, D), u32),
            pltpu.VMEM((NTILES * HQ, 512), u32),
            pltpu.VMEM((NTILES, D, TQ), bf16),
            pltpu.VMEM((NQ * HQ, D), u32),
            pltpu.VMEM((NQ * HQ, 512), u32),
            pltpu.VMEM((NQ, D, TQ), f32),
            pltpu.VMEM((TQ, D), bf16),
            pltpu.VMEM((HQ, D), u32),
        ],
        compiler_params=pltpu.CompilerParams(
            dimension_semantics=("arbitrary",),
            vmem_limit_bytes=64 * 1024 * 1024,
        ),
    )(A_x.reshape(S, D), A_wqkv, A_wo, B_w1, B_b1, B_w2, B_b2)
    return out.reshape(1, S, D)
```
